```python
import os as _os
_os.environ.setdefault("JAX_PLATFORMS", "cpu")
import jax
import jax.numpy as jnp

def _softmax(x, axis=-1):
    return jax.nn.softmax(x, axis=axis)
def _gelu(x):
    return jax.nn.gelu(x, approximate=True)
def _silu(x):
    return jax.nn.silu(x)
def _sigmoid(x):
    return jax.nn.sigmoid(x)
def _layernorm(x, axis=-1, eps=1e-5):
    m = jnp.mean(x, axis=axis, keepdims=True)
    v = jnp.var(x, axis=axis, keepdims=True)
    return (x - m) / jnp.sqrt(v + eps)
def _scatter_add(tgt, idx, src, axis=0):
    return tgt.at[idx].add(src)
def _segment_sum(src, seg, n):
    return jax.ops.segment_sum(src, seg, n)
class _Rng:
    def __init__(self, key):
        self._k = key
    def _next(self):
        self._k, sub = jax.random.split(self._k)
        return sub
    def normal(self, shape):
        return jax.random.normal(self._next(), shape, dtype=jnp.bfloat16)
    def randint(self, lo, hi, shape):
        return jax.random.randint(self._next(), shape, lo, hi, dtype=jnp.int32)
    def uniform(self, shape, lo=0.0, hi=1.0):
        return jax.random.uniform(self._next(), shape, jnp.bfloat16, lo, hi)
    def permutation(self, n):
        return jax.random.permutation(self._next(), n)


kernel_name = 'standalone__gqa_block_cached__near_ridge'

def setup_inputs():
    _rng = _Rng(jax.random.key(int.from_bytes(__import__("os").urandom(4), "little")))
    _w = (lambda a: (lambda t: t.astype(jnp.bfloat16) if jnp.issubdtype(t.dtype, jnp.floating) else t)(jnp.asarray(a)))
    B, Sq, D = 8, 64, 512
    Hq, Hkv, Sk, Dh = 32, 8, 64, 128
    assert Hq % Hkv == 0, (Hq, Hkv)
    return {
        "x": _w((lambda *s: _rng.normal(s) * 0.8)(B, Sq, D)),
        "k_cache": _w((lambda *s: _rng.normal(s) * 0.8)(B, Hkv, Sk, Dh)),
        "v_cache": _w((lambda *s: _rng.normal(s) * 0.05)(B, Hkv, Sk, Dh)),
        "wq": _w((lambda *s: _rng.normal(s) * 0.8)(D, Hq * Dh) * (D ** -0.5)),
        "wo": _w((lambda *s: _rng.normal(s) * 0.05)(Hq * Dh, D) * ((Hq * Dh) ** -0.5)),
    }

def reference(x, k_cache, v_cache, wq, wo):
    B, Sq, D = x.shape
    Hq, Dh = 32, 128
    Hkv = k_cache.shape[1]
    rep = Hq // Hkv
    q = (lambda x, *d: x.transpose(*d))((x @ wq).reshape(B, Sq, Hq, Dh), 0, 2, 1, 3)
    k = jnp.repeat(k_cache, rep, axis=1)
    v = jnp.repeat(v_cache, rep, axis=1)
    scores = jnp.einsum("bhqd,bhkd->bhqk", q, k) * (Dh ** -0.5)
    p = _softmax(scores, axis=-1)
    o = jnp.einsum("bhqk,bhkd->bhqd", p, v)
    return (lambda x, *d: x.transpose(*d))(o, 0, 2, 1, 3).reshape(B, Sq, Hq * Dh) @ wo
```

```python
import functools
import jax, jax.numpy as jnp
from jax import lax
import jax.experimental.pallas as pl
import jax.experimental.pallas.tpu as pltpu
import numpy as np

NT = (((1,), (1,)), ((), ()))
C = float(128 ** -0.5 * np.log2(np.e))
ANY = pl.BlockSpec(memory_space=pl.ANY)
f32, bf16, u32 = jnp.float32, jnp.bfloat16, jnp.uint32

def make(order='SHP', pv_split=2, approx=True, vmem=100):
    def kern(x_hbm, k_hbm, v_hbm, wq_hbm, wo_hbm, out_hbm,
             xb, kb, vb, wqb, wob, q_scr, o_scr, acc, ob, sems):
        cp_x = pltpu.make_async_copy(x_hbm, xb, sems.at[0])
        cp_wq = [pltpu.make_async_copy(wq_hbm.at[:, pl.ds(g*512, 512)], wqb.at[g], sems.at[1+g]) for g in range(8)]
        cp_wo = [pltpu.make_async_copy(wo_hbm.at[pl.ds(g*512, 512), :], wob.at[g], sems.at[9+g]) for g in range(8)]
        cp_k = [pltpu.make_async_copy(k_hbm.at[:, g], kb.at[g], sems.at[17+g]) for g in range(8)]
        cp_v = [pltpu.make_async_copy(v_hbm.at[:, g], vb.at[g], sems.at[25+g]) for g in range(8)]
        cp_x.start(); cp_wq[0].start()
        for g in range(8):
            if g + 1 < 8: cp_wq[g+1].start()
            cp_k[g].start(); cp_v[g].start(); cp_wo[g].start()

        def qproj(g, j):
            q = jnp.dot(xb[...], wqb[g, :, j*128:(j+1)*128], preferred_element_type=f32)
            q_scr[g % 2, j] = pltpu.bitcast(q.astype(bf16), u32)

        def scores(g, b):
            qs = jnp.concatenate([pltpu.bitcast(q_scr[g % 2, h, b*32:(b+1)*32, :], bf16) for h in range(4)], axis=0)
            st = lax.dot_general(kb[g, b], qs, NT, preferred_element_type=f32)
            m = jnp.max(st, axis=0, keepdims=True)
            p = jnp.exp2((st - m) * C)
            l = jnp.sum(p, axis=0, keepdims=True)
            r = pl.reciprocal(l, approx=True) if approx else 1.0 / l
            return (p * r).astype(bf16).T

        def pv(g, b, p):
            vv = vb[g, b]
            n = 4 // pv_split
            for s in range(pv_split):
                o = jnp.dot(p[s*n*64:(s+1)*n*64], vv, preferred_element_type=f32).astype(bf16)
                for hh in range(n):
                    h = s*n + hh
                    o_scr[g % 2, h, b*32:(b+1)*32, :] = pltpu.bitcast(o[hh*64:(hh+1)*64], u32)

        def oproj(g, j):
            o = jnp.concatenate([pltpu.bitcast(o_scr[g % 2, h], bf16) for h in range(4)], axis=1)
            y = jnp.dot(o, wob[g, :, j*128:(j+1)*128], preferred_element_type=f32)
            if g == 0:
                acc[:, j*128:(j+1)*128] = y
            elif g < 7:
                acc[:, j*128:(j+1)*128] += y
            else:
                ob[:, j*128:(j+1)*128] = (acc[:, j*128:(j+1)*128] + y).astype(bf16)

        cp_x.wait(); cp_wq[0].wait()
        for j in range(4): qproj(0, j)
        for g in range(8):
            heavy = []
            if g >= 1:
                cp_wo[g-1].wait()
                heavy += [functools.partial(oproj, g-1, j) for j in range(4)]
            if g + 1 < 8:
                cp_wq[g+1].wait()
                heavy = [functools.partial(qproj, g+1, j) for j in range(4)] + heavy
            cp_k[g].wait(); cp_v[g].wait()
            per = max(1, len(heavy) // 8)
            hi = 0
            for b in range(8):
                if order == 'SHP':
                    p = scores(g, b)
                    for _ in range(per):
                        if hi < len(heavy): heavy[hi](); hi += 1
                    pv(g, b, p)
                elif order == 'SPH':
                    p = scores(g, b); pv(g, b, p)
                    for _ in range(per):
                        if hi < len(heavy): heavy[hi](); hi += 1
            while hi < len(heavy): heavy[hi](); hi += 1
        cp_wo[7].wait()
        for j in range(4): oproj(7, j)
        cp_o = pltpu.make_async_copy(ob, out_hbm, sems.at[33]); cp_o.start(); cp_o.wait()

    def fn(x, k, v, wq, wo):
        out = pl.pallas_call(
            kern,
            in_specs=[ANY]*5, out_specs=ANY,
            out_shape=jax.ShapeDtypeStruct((512, 512), bf16),
            scratch_shapes=[
                pltpu.VMEM((512, 512), bf16),
                pltpu.VMEM((8, 8, 64, 128), bf16),
                pltpu.VMEM((8, 8, 64, 128), bf16),
                pltpu.VMEM((8, 512, 512), bf16),
                pltpu.VMEM((8, 512, 512), bf16),
                pltpu.VMEM((2, 4, 256, 128), u32),
                pltpu.VMEM((2, 4, 256, 128), u32),
                pltpu.VMEM((512, 512), f32),
                pltpu.VMEM((512, 512), bf16),
                pltpu.SemaphoreType.DMA((34,)),
            ],
            compiler_params=pltpu.CompilerParams(vmem_limit_bytes=vmem*2**20),
        )(x.reshape(512, 512), k, v, wq, wo)
        return out.reshape(8, 64, 512)
    return fn


_impl = make('SHP', 2)


@jax.jit
def pallas_standalone__gqa_block_cached__near_ridge_kernel(x, k_cache, v_cache, wq, wo):
    return _impl(x, k_cache, v_cache, wq, wo)
```

```python
import functools
import jax, jax.numpy as jnp
from jax import lax
import jax.experimental.pallas as pl
import jax.experimental.pallas.tpu as pltpu
import numpy as np

NT = (((1,), (1,)), ((), ()))
C = float(128 ** -0.5 * np.log2(np.e))
ANY = pl.BlockSpec(memory_space=pl.ANY)
f32, bf16, u32 = jnp.float32, jnp.bfloat16, jnp.uint32

def build(plan, pv_split=2, vmem=100, **cparams):
    names = []
    for op in plan:
        if op[0] == 'S': names.append(op[1])
    assert len(set(names)) == len(names)
    sid = {n: i for i, n in enumerate(names)}
    def kern(x_hbm, k_hbm, v_hbm, wq_hbm, wo_hbm, out_hbm, xb, kb, vb, wqb, wob, ob, sems):
        def desc(it):
            t = it[0]
            if t == 'x':
                sl = pl.ds(it[1]*128, (it[2]-it[1])*128); return (x_hbm.at[:, sl], xb.at[:, sl])
            if t == 'wq':
                r = pl.ds(it[1]*128, (it[2]-it[1])*128); c = pl.ds(it[3]*512, (it[4]-it[3])*512)
                return (wq_hbm.at[r, c], wqb.at[r, c])
            if t == 'wqh':
                c = pl.ds(it[1]*128, (it[2]-it[1])*128); return (wq_hbm.at[:, c], wqb.at[:, c])
            if t == 'kk':
                s = pl.ds(it[1], it[2]-it[1]); return (k_hbm.at[:, s], kb.at[:, s])
            if t == 'vv':
                s = pl.ds(it[1], it[2]-it[1]); return (v_hbm.at[:, s], vb.at[:, s])
            if t == 'wo':
                r = pl.ds(it[1]*512, (it[2]-it[1])*512); return (wo_hbm.at[r, :], wob.at[r, :])
            if t == 'out':
                r = pl.ds(it[1]*64, (it[2]-it[1])*64); return (ob.at[r, :], out_hbm.at[r, :])
        def cp(it):
            s, d = desc(it); return pltpu.make_async_copy(s, d, sems.at[sid[it]])
        Q = {}; O = {}; P = {}; ACC = {}
        def qproj(g, j):
            c = g*512 + j*128
            Q[g, j] = jnp.dot(xb[...], wqb[:, c:c+128], preferred_element_type=f32)
        def qproj_k(g, k0, k1):
            for j in range(4):
                c = g*512 + j*128
                y = jnp.dot(xb[:, k0*128:k1*128], wqb[k0*128:k1*128, c:c+128], preferred_element_type=f32)
                Q[g, j] = y if k0 == 0 else y + Q[g, j]
        def scores(g, b):
            qs = jnp.concatenate([Q[g, h][b*64:(b+1)*64] for h in range(4)], axis=0).astype(bf16)
            st = lax.dot_general(kb[b, g], qs, NT, preferred_element_type=f32)
            m = jnp.max(st, axis=0, keepdims=True)
            p = jnp.exp2((st - m) * C)
            l = jnp.sum(p, axis=0, keepdims=True)
            P[g, b] = (p * pl.reciprocal(l, approx=True)).astype(bf16).T
        def pv(g, b):
            p = P.pop((g, b)); vv = vb[b, g]
            n = 4 // pv_split
            for s in range(pv_split):
                o = jnp.dot(p[s*n*64:(s+1)*n*64], vv, preferred_element_type=f32)
                for hh in range(n):
                    O[g, b, s*n + hh] = o[hh*64:(hh+1)*64]
        def olhs(g, b0, b1):
            key = ('lhs', g, b0, b1)
            if key not in O:
                O[key] = jnp.concatenate([jnp.concatenate([O[g, b, h] for b in range(b0, b1)], axis=0) for h in range(4)], axis=1).astype(bf16)
            return O[key]
        def oproj(g, j):
            y = jnp.dot(olhs(g, 0, 8), wob[g*512:(g+1)*512, j*128:(j+1)*128], preferred_element_type=f32)
            ACC[j] = y if j not in ACC else y + ACC[j]
        def oproj_m(gs, b0, b1):
            for j in range(4):
                tot = ACC[j][b0*64:b1*64] if j in ACC else None
                for g in gs:
                    y = jnp.dot(olhs(g, b0, b1), wob[g*512:(g+1)*512, j*128:(j+1)*128], preferred_element_type=f32)
                    tot = y if tot is None else y + tot
                ob[b0*64:b1*64, j*128:(j+1)*128] = tot.astype(bf16)
        for op in plan:
            t = op[0]
            if t == 'S': pltpu.async_copy(*desc(op[1]), sems.at[sid[op[1]]], priority=(op[2] if len(op) > 2 else 0))
            elif t == 'W': cp(op[1]).wait()
            elif t == 'qk': qproj_k(*op[1:])
            elif t == 'q': qproj(*op[1:])
            elif t == 's': scores(*op[1:])
            elif t == 'p': pv(*op[1:])
            elif t == 'o': oproj(*op[1:])
            elif t == 'om': oproj_m(*op[1:])
            else: raise ValueError(op)

    def fn(x, k, v, wq, wo):
        out = pl.pallas_call(
            kern,
            in_specs=[ANY]*5, out_specs=ANY,
            out_shape=jax.ShapeDtypeStruct((512, 512), bf16),
            scratch_shapes=[
                pltpu.VMEM((512, 512), bf16), pltpu.VMEM((8, 8, 64, 128), bf16), pltpu.VMEM((8, 8, 64, 128), bf16),
                pltpu.VMEM((512, 4096), bf16), pltpu.VMEM((4096, 512), bf16),
                pltpu.VMEM((512, 512), bf16),
                pltpu.SemaphoreType.DMA((len(names),)),
            ],
            compiler_params=pltpu.CompilerParams(vmem_limit_bytes=vmem*2**20, **cparams),
        )(x.reshape(512, 512), k, v, wq, wo)
        return out.reshape(8, 64, 512)
    return fn

def Qs(g): return [('q', g, j) for j in range(4)]
def Os(g): return [('o', g, j) for j in range(4)]
def mix(units, heavy):
    out = []
    n, m = len(units), len(heavy)
    if n == 0: return list(heavy)
    if m == 0:
        return [(t, g, b) for (g, b) in units for t in 'sp']
    if m >= n:
        for i, u in enumerate(units):
            hs = heavy[i*m//n:(i+1)*m//n]
            out += [('s',) + u] + list(hs) + [('p',) + u]
    else:
        for i, h in enumerate(heavy):
            us = units[i*n//m:(i+1)*n//m]
            out += [('s',) + u for u in us] + [h] + [('p',) + u for u in us]
    return out
def A(g): return [(g, b) for b in range(8)]
def tail(gs, chunks):
    p = []
    for (b0, b1) in chunks:
        p += [('om', tuple(gs), b0, b1), ('S', ('out', b0, b1))]
    p += [('W', ('out', b0, b1)) for (b0, b1) in chunks]
    return p
def SW(items, prio=0): return [('S', i, prio) for i in items]
def WW(items): return [('W', i) for i in items]
wq = lambda g0, g1=None: ('wq', 0, 4, g0, g0+1 if g1 is None else g1)
wo = lambda g0, g1=None: ('wo', g0, g0+1 if g1 is None else g1)
kv = lambda g0, g1=None: [('kk', g0, g0+1 if g1 is None else g1), ('vv', g0, g0+1 if g1 is None else g1)]

def plan_5bar(out_chunks=((0,2),(2,4),(4,6),(6,8))):
    X = ('x', 0, 4)
    b0 = [X, wq(0)]; b1 = [wq(1), wq(2)]; b2 = kv(0, 2) + [wq(3), wq(4), wo(0)]
    b3 = kv(2, 4) + [wq(5), wq(6), wo(1)]; b4 = kv(4, 8) + [wq(7)] + [wo(g) for g in range(2, 8)]
    p = SW(b0 + b1 + b2 + b3 + b4)
    p += WW(b0) + Qs(0)
    p += WW(b1) + Qs(1) + Qs(2)
    p += WW(b2) + mix(A(0) + A(1), Qs(3) + Qs(4) + Os(0))
    p += WW(b3) + mix(A(2) + A(3), Qs(5) + Qs(6) + Os(1))
    p += WW(b4) + mix(A(4), Qs(7) + Os(2)) + mix(A(5), Os(3)) + mix(A(6), Os(4)) + mix(A(7), Os(5)) + Os(6)
    p += tail([7], out_chunks)
    return p

RD = {'XLA_TPU_RESCHEDULE_DMA_DONES': True}

def plan_phase(kch=((0,4),), out_chunks=((0,2),(2,4),(4,6),(6,8)), last=7, start_all=True, qfirst=True):
    items = []
    for (k0, k1) in kch:
        items += [('x', k0, k1), ('wq', k0, k1, 0, 1)]
    rest = []
    for g in range(8):
        if g + 1 < 8: rest += [wq(g+1)]
        rest += kv(g)
        if g >= 1: rest += [wo(g-1)]
    rest += [wo(7)]
    p = SW(items + rest)
    if len(kch) == 1:
        p += WW(items) + Qs(0)
    else:
        for (k0, k1) in kch:
            p += WW([('x', k0, k1), ('wq', k0, k1, 0, 1)]) + [('qk', 0, k0, k1)]
    for g in range(8):
        qh = ([('W', wq(g+1))] + Qs(g+1)) if g + 1 < 8 else []
        oh = ([('W', wo(g-1))] + Os(g-1)) if g >= 1 else []
        def fold(l): return ([l[0:2]] + [[o] for o in l[2:]]) if l else []
        heavy = (fold(qh) + fold(oh)) if qfirst else (fold(oh) + fold(qh))
        m = mix(A(g), heavy)
        flat = []
        for o in m:
            flat += o if isinstance(o, list) else [o]
        p += WW(kv(g)) + flat
    p += [('W', wo(7))] + tail([7], out_chunks)
    return p

def auto_start(plan, depth, first=None):
    items = [op[1] for op in plan if op[0] == 'W' and op[1][0] != 'out']
    first = depth if first is None else first
    out = [('S', it) for it in items[:first]]
    nxt = first; seen = 0
    for op in plan:
        out.append(op)
        if op[0] == 'W' and op[1][0] != 'out':
            seen += 1
            while nxt < len(items) and nxt < seen + depth:
                out.append(('S', items[nxt])); nxt += 1
    return out

def wqh(g, j): return ('wqh', g*4 + j, g*4 + j + 1)

def plan_fine(kch=((0,1),(1,2),(2,3),(3,4)), out_chunks=((0,4),(4,6),(6,7),(7,8)), depth=6, first=None, head_groups=(1,), wfirst=True, qfirst=True):
    p = []
    for (k0, k1) in kch:
        its = [('wq', k0, k1, 0, 1), ('x', k0, k1)] if wfirst else [('x', k0, k1), ('wq', k0, k1, 0, 1)]
        p += WW(its) + [('qk', 0, k0, k1)]
    for g in range(8):
        if g + 1 < 8:
            if g + 1 in head_groups:
                qh = [[('W', wqh(g+1, j)), ('q', g+1, j)] for j in range(4)]
            else:
                qh = [[('W', wq(g+1)), ('q', g+1, 0)]] + [[('q', g+1, j)] for j in range(1, 4)]
        else: qh = []
        oh = ([[('W', wo(g-1)), ('o', g-1, 0)]] + [[('o', g-1, j)] for j in range(1, 4)]) if g >= 1 else []
        heavy = (qh + oh) if qfirst else (oh + qh)
        flat = []
        for o in mix(A(g), heavy): flat += o if isinstance(o, list) else [o]
        if g == 0 and 1 in head_groups:
            pass
        p += WW(kv(g)) + flat
    p += [('W', wo(7))] + tail([7], out_chunks)
    return auto_start(p, depth, first)
FL = dict(flags=RD, disable_semaphore_checks=True)


_impl = build(plan_fine(depth=6), **FL)


@jax.jit
def pallas_standalone__gqa_block_cached__near_ridge_kernel(x, k_cache, v_cache, wq, wo):
    return _impl(x, k_cache, v_cache, wq, wo)
```

```python
import jax
import jax.numpy as jnp
import numpy as np
from jax import lax
import jax.experimental.pallas as pl
import jax.experimental.pallas.tpu as pltpu

B, SQ, D = 8, 64, 512
HQ, HKV, SK, DH = 32, 8, 64, 128
REP = HQ // HKV
GW = REP * DH
T = 128
NKT = D // T
NNT = D // T
LOG2E_SCALE = float(DH ** -0.5 * np.log2(np.e))

F32, BF16 = jnp.float32, jnp.bfloat16
_NT_DIMS = (((1,), (1,)), ((), ()))

Q_AHEAD = 2
DMA_AHEAD = 10

_WHOLE = ((0, 8),)
_HALVES = ((0, 4), (4, 8))
_QUARTERS = ((0, 2), (2, 4), (4, 6), (6, 8))
_FINE = ((0, 2), (2, 4), (4, 5), (5, 6), (6, 7), (7, 8))
START_ROWS = {(0, 0): _FINE, (0, 1): _QUARTERS, (1, 0): _QUARTERS, (1, 1): _QUARTERS,
              (2, 0): _QUARTERS}
X_ROWS = {0: _FINE, 1: _HALVES, 2: _HALVES, 3: _WHOLE}
X_BEFORE_WQ = (1, 2)
WQ_BY_HEAD = (Q_AHEAD,)
OUT_PIECES = ((0, 2, 0, 4), (2, 4, 0, 4), (4, 6, 0, 4), (6, 8, 0, 2), (6, 8, 2, 3),
              (6, 7, 3, 4), (7, 8, 3, 4))


def _interleave(units, heavy):
    steps, n, m = [], len(units), len(heavy)
    if m >= n:
        for i, u in enumerate(units):
            mid = [op for h in heavy[i * m // n:(i + 1) * m // n] for op in h]
            steps += [("scores",) + u] + mid + [("pv",) + u]
    else:
        for i, h in enumerate(heavy):
            us = units[i * n // m:(i + 1) * n // m]
            steps += [("scores",) + u for u in us] + list(h) + [("pv",) + u for u in us]
    return steps


def _build_schedule():
    steps = []
    all_heads = tuple(range(REP))

    for kt in range(NKT):
        for g in range(Q_AHEAD):
            wq_wait = ("wait", ("wq", kt, kt + 1, REP * g, REP * (g + 1)))
            x_rows = list(X_ROWS[kt]) if g == 0 else []
            if not (g == 0 and kt in X_BEFORE_WQ):
                steps.append(wq_wait)
                wq_wait = None
            for lo, hi in START_ROWS.get((kt, g), _WHOLE):
                while x_rows and x_rows[0][0] < hi:
                    r0, r1 = x_rows.pop(0)
                    steps.append(("wait", ("x", kt, kt + 1, r0, r1)))
                if wq_wait is not None:
                    steps.append(wq_wait)
                    wq_wait = None
                steps.append(("qproj", g, all_heads, kt, kt + 1, lo, hi))

    for g in range(HKV):
        heavy = []
        gq = g + Q_AHEAD
        if gq < HKV:
            qp = [("qproj", gq, (j,), 0, NKT, 0, B) for j in range(REP)]
            if gq in WQ_BY_HEAD:
                heavy += [[("wait", ("wq", 0, NKT, REP * gq + j, REP * gq + j + 1)), qp[j]]
                          for j in range(REP)]
            else:
                heavy += [[("wait", ("wq", 0, NKT, REP * gq, REP * (gq + 1))), qp[0]]]
                heavy += [[op] for op in qp[1:]]
        if g >= 1:
            heavy += [[("wait", ("wo", g - 1)), ("oproj", g - 1, 0)]]
            heavy += [[("oproj", g - 1, j)] for j in range(1, NNT)]
        body = _interleave([(g, b) for b in range(B)], heavy)
        first_pv = [i for i, op in enumerate(body) if op[0] == "pv"][0]
        steps += [("wait", ("k", g))] + body[:first_pv] + [("wait", ("v", g))] + body[first_pv:]

    steps.append(("wait", ("wo", HKV - 1)))
    for piece in OUT_PIECES:
        steps += [("ofinal", HKV - 1) + piece, ("start", ("out",) + piece)]
    steps += [("wait", ("out",) + piece) for piece in OUT_PIECES]

    inputs = [op[1] for op in steps if op[0] == "wait" and op[1][0] != "out"]
    paced = [("start", it) for it in inputs[:DMA_AHEAD]]
    nxt = DMA_AHEAD
    for op in steps:
        paced.append(op)
        if op[0] == "wait" and op[1][0] != "out" and nxt < len(inputs):
            paced.append(("start", inputs[nxt]))
            nxt += 1
    return tuple(paced)


_SCHEDULE = _build_schedule()
_COPIES = tuple(op[1] for op in _SCHEDULE if op[0] == "start")
_SEM_OF = {it: i for i, it in enumerate(_COPIES)}


def _kernel(x_hbm, k_hbm, v_hbm, wq_hbm, wo_hbm, out_hbm,
            x_vm, k_vm, v_vm, wq_vm, wo_vm, out_vm, sems):

    def copy(item):
        kind = item[0]
        if kind == "x":
            _, k0, k1, r0, r1 = item
            idx = (pl.ds(r0 * SQ, (r1 - r0) * SQ), pl.ds(k0 * T, (k1 - k0) * T))
            src, dst = x_hbm.at[idx], x_vm.at[idx]
        elif kind == "wq":
            _, k0, k1, h0, h1 = item
            idx = (pl.ds(k0 * T, (k1 - k0) * T), pl.ds(h0 * DH, (h1 - h0) * DH))
            src, dst = wq_hbm.at[idx], wq_vm.at[idx]
        elif kind == "k":
            idx = (slice(None), pl.ds(item[1], 1))
            src, dst = k_hbm.at[idx], k_vm.at[idx]
        elif kind == "v":
            idx = (slice(None), pl.ds(item[1], 1))
            src, dst = v_hbm.at[idx], v_vm.at[idx]
        elif kind == "wo":
            idx = (pl.ds(item[1] * GW, GW), slice(None))
            src, dst = wo_hbm.at[idx], wo_vm.at[idx]
        else:
            _, r0, r1, c0, c1 = item
            idx = (pl.ds(r0 * SQ, (r1 - r0) * SQ), pl.ds(c0 * T, (c1 - c0) * T))
            src, dst = out_vm.at[idx], out_hbm.at[idx]
        return pltpu.make_async_copy(src, dst, sems.at[_SEM_OF[item]])

    q_full, q_rows = {}, {}
    probs = {}
    attn = {}
    attn_lhs = {}
    acc = {}

    def qproj(g, heads, k0, k1, b0, b1):
        lhs = x_vm[b0 * SQ:b1 * SQ, k0 * T:k1 * T]
        for h in heads:
            col = g * GW + h * DH
            y = jnp.dot(lhs, wq_vm[k0 * T:k1 * T, col:col + DH], preferred_element_type=F32)
            if (b0, b1) == (0, B):
                if k0 != 0:
                    if (g, h) not in q_full:
                        q_full[g, h] = jnp.concatenate(
                            [q_rows.pop((g, h, b)) for b in range(B)], axis=0)
                    y = y + q_full[g, h]
                q_full[g, h] = y
            else:
                if k0 != 0 and (g, h) in q_full:
                    whole = q_full.pop((g, h))
                    for b in range(B):
                        q_rows[g, h, b] = whole[b * SQ:(b + 1) * SQ]
                for b in range(b0, b1):
                    part = y[(b - b0) * SQ:(b - b0 + 1) * SQ]
                    q_rows[g, h, b] = part if k0 == 0 else part + q_rows[g, h, b]

    def scores(g, b):
        def q_of(h):
            return q_full[g, h][b * SQ:(b + 1) * SQ] if (g, h) in q_full else q_rows[g, h, b]
        q = jnp.concatenate([q_of(h) for h in range(REP)], axis=0).astype(BF16)
        st = lax.dot_general(k_vm[b, g], q, _NT_DIMS, preferred_element_type=F32)
        m = jnp.max(st, axis=0, keepdims=True)
        e = jnp.exp2((st - m) * LOG2E_SCALE)
        inv = 1.0 / jnp.sum(e, axis=0, keepdims=True)
        probs[g, b] = (e * inv).astype(BF16).T

    def pv(g, b):
        p, v = probs.pop((g, b)), v_vm[b, g]
        half = REP // 2
        for s in range(2):
            o = jnp.dot(p[s * half * SQ:(s + 1) * half * SQ], v, preferred_element_type=F32)
            for i in range(half):
                attn[g, b, s * half + i] = o[i * SQ:(i + 1) * SQ]

    def out_lhs(g, b0, b1):
        if (g, b0, b1) not in attn_lhs:
            cols = [jnp.concatenate([attn[g, b, h] for b in range(b0, b1)], axis=0)
                    for h in range(REP)]
            attn_lhs[g, b0, b1] = jnp.concatenate(cols, axis=1).astype(BF16)
        return attn_lhs[g, b0, b1]

    def wo_tile(g, j):
        return wo_vm[g * GW:(g + 1) * GW, j * T:(j + 1) * T]

    def oproj(g, j):
        y = jnp.dot(out_lhs(g, 0, B), wo_tile(g, j), preferred_element_type=F32)
        acc[j] = y if j not in acc else y + acc[j]

    def ofinal(g, b0, b1, j0, j1):
        for j in range(j0, j1):
            y = jnp.dot(out_lhs(g, b0, b1), wo_tile(g, j), preferred_element_type=F32)
            total = y + acc[j][b0 * SQ:b1 * SQ]
            out_vm[b0 * SQ:b1 * SQ, j * T:(j + 1) * T] = total.astype(BF16)

    emit = {"start": lambda item: copy(item).start(), "wait": lambda item: copy(item).wait(),
            "qproj": qproj, "scores": scores, "pv": pv, "oproj": oproj, "ofinal": ofinal}
    for step in _SCHEDULE:
        emit[step[0]](*step[1:])


def _compiler_params():
    params = dict(vmem_limit_bytes=64 * 1024 * 1024)
    if jax.__version_info__ >= (0, 12):
        params.update(flags={"XLA_TPU_RESCHEDULE_DMA_DONES": True}, disable_semaphore_checks=True)
    return pltpu.CompilerParams(**params)


@jax.jit
def pallas_standalone__gqa_block_cached__near_ridge_kernel(
    x: jax.Array,
    k_cache: jax.Array,
    v_cache: jax.Array,
    wq: jax.Array,
    wo: jax.Array,
):
    assert x.shape == (B, SQ, D), x.shape
    assert k_cache.shape == v_cache.shape == (B, HKV, SK, DH), (k_cache.shape, v_cache.shape)
    assert wq.shape == (D, HQ * DH) and wo.shape == (HQ * DH, D), (wq.shape, wo.shape)

    any_space = pl.BlockSpec(memory_space=pl.ANY)
    out = pl.pallas_call(
        _kernel,
        in_specs=[any_space] * 5,
        out_specs=any_space,
        out_shape=jax.ShapeDtypeStruct((B * SQ, D), x.dtype),
        scratch_shapes=[
            pltpu.VMEM((B * SQ, D), x.dtype),
            pltpu.VMEM((B, HKV, SK, DH), k_cache.dtype),
            pltpu.VMEM((B, HKV, SK, DH), v_cache.dtype),
            pltpu.VMEM((D, HQ * DH), wq.dtype),
            pltpu.VMEM((HQ * DH, D), wo.dtype),
            pltpu.VMEM((B * SQ, D), x.dtype),
            pltpu.SemaphoreType.DMA((len(_COPIES),)),
        ],
        compiler_params=_compiler_params(),
    )(x.reshape(B * SQ, D), k_cache, v_cache, wq, wo)
    return out.reshape(B, SQ, D)
```

```python
import jax
import jax.numpy as jnp
import numpy as np
from jax import lax
import jax.experimental.pallas as pl
import jax.experimental.pallas.tpu as pltpu

B, SQ, D = 8, 64, 512
HQ, HKV, SK, DH = 32, 8, 64, 128
REP = HQ // HKV
GW = REP * DH
T = 128
NKT = D // T
NNT = D // T
LOG2E_SCALE = float(DH ** -0.5 * np.log2(np.e))

F32, BF16 = jnp.float32, jnp.bfloat16
_NT_DIMS = (((1,), (1,)), ((), ()))

Q_AHEAD = 2
DMA_AHEAD = 14

_WHOLE = ((0, 8),)
_HALVES = ((0, 4), (4, 8))
_QUARTERS = ((0, 2), (2, 4), (4, 6), (6, 8))
_THIRDS = ((0, 4), (4, 6), (6, 8))
_FINE = ((0, 2), (2, 4), (4, 6), (6, 7), (7, 8))
START_ROWS = {(0, 0): _FINE, (0, 1): _FINE, (1, 0): _QUARTERS, (1, 1): _QUARTERS,
              (2, 0): _THIRDS, (2, 1): _FINE, (3, 0): _QUARTERS}
X_ROWS = {0: _FINE, 1: _HALVES, 2: _HALVES, 3: _WHOLE}
WQ_BY_HEAD = (Q_AHEAD,)
OUT_PIECES = ((0, 2, 0, 4), (2, 4, 0, 4), (4, 6, 0, 4), (6, 7, 0, 4),
              (7, 8, 0, 2), (7, 8, 2, 3), (7, 8, 3, 4))


def _interleave(units, heavy):
    steps = []
    if len(heavy) == len(units):
        for u, h in zip(units, heavy):
            steps += [("scores",) + u] + h + [("pv",) + u]
    else:
        assert 2 * len(heavy) == len(units)
        pending = []
        for i, h in enumerate(heavy):
            pair = units[2 * i:2 * i + 2]
            steps += [("scores",) + u for u in pair] + [("pv",) + u for u in pending] + h
            pending = pair
        steps += [("pv",) + u for u in pending]
    return steps


def _build_schedule():
    steps = []
    all_heads = tuple(range(REP))

    for kt in range(NKT):
        for g in range(Q_AHEAD):
            steps.append(("wait", ("wq", kt, kt + 1, REP * g, REP * (g + 1))))
            x_rows = list(X_ROWS[kt]) if g == 0 else []
            for lo, hi in START_ROWS.get((kt, g), _WHOLE):
                while x_rows and x_rows[0][0] < hi:
                    r0, r1 = x_rows.pop(0)
                    steps.append(("wait", ("x", kt, kt + 1, r0, r1)))
                steps.append(("qproj", g, all_heads, kt, kt + 1, lo, hi))

    for g in range(HKV):
        heavy = []
        gq = g + Q_AHEAD
        if gq < HKV:
            qp = [("qproj", gq, (j,), 0, NKT, 0, B) for j in range(REP)]
            if gq in WQ_BY_HEAD:
                heavy += [[("wait", ("wq", 0, NKT, REP * gq + j, REP * gq + j + 1)), qp[j]]
                          for j in range(REP)]
            else:
                heavy += [[("wait", ("wq", 0, NKT, REP * gq, REP * (gq + 1))), qp[0]]]
                heavy += [[op] for op in qp[1:]]
        if g >= 1:
            heavy += [[("wait", ("wo", g - 1)), ("oproj", g - 1, 0)]]
            heavy += [[("oproj", g - 1, j)] for j in range(1, NNT)]
        body = _interleave([(g, b) for b in range(B)], heavy)
        first_pv = [i for i, op in enumerate(body) if op[0] == "pv"][0]
        steps += [("wait", ("k", g))] + body[:first_pv] + [("wait", ("v", g))] + body[first_pv:]

    steps.append(("wait", ("wo", HKV - 1)))
    for piece in OUT_PIECES:
        steps += [("ofinal", HKV - 1) + piece, ("start", ("out",) + piece)]
    steps += [("wait", ("out",) + piece) for piece in OUT_PIECES]

    inputs = [op[1] for op in steps if op[0] == "wait" and op[1][0] != "out"]
    paced = [("start", it) for it in inputs[:DMA_AHEAD]]
    nxt = DMA_AHEAD
    for op in steps:
        paced.append(op)
        if op[0] == "wait" and op[1][0] != "out" and nxt < len(inputs):
            paced.append(("start", inputs[nxt]))
            nxt += 1
    return tuple(paced)


_SCHEDULE = _build_schedule()
_COPIES = tuple(op[1] for op in _SCHEDULE if op[0] == "start")
_SEM_OF = {it: i for i, it in enumerate(_COPIES)}


def _kernel(x_hbm, k_hbm, v_hbm, wq_hbm, wo_hbm, out_hbm,
            x_vm, k_vm, v_vm, wq_vm, wo_vm, out_vm, sems):

    def copy(item):
        kind = item[0]
        if kind == "x":
            _, k0, k1, r0, r1 = item
            idx = (pl.ds(r0 * SQ, (r1 - r0) * SQ), pl.ds(k0 * T, (k1 - k0) * T))
            src, dst = x_hbm.at[idx], x_vm.at[idx]
        elif kind == "wq":
            _, k0, k1, h0, h1 = item
            idx = (pl.ds(k0 * T, (k1 - k0) * T), pl.ds(h0 * DH, (h1 - h0) * DH))
            src, dst = wq_hbm.at[idx], wq_vm.at[idx]
        elif kind == "k":
            idx = (slice(None), pl.ds(item[1], 1))
            src, dst = k_hbm.at[idx], k_vm.at[idx]
        elif kind == "v":
            idx = (slice(None), pl.ds(item[1], 1))
            src, dst = v_hbm.at[idx], v_vm.at[idx]
        elif kind == "wo":
            idx = (pl.ds(item[1] * GW, GW), slice(None))
            src, dst = wo_hbm.at[idx], wo_vm.at[idx]
        else:
            _, r0, r1, c0, c1 = item
            idx = (pl.ds(r0 * SQ, (r1 - r0) * SQ), pl.ds(c0 * T, (c1 - c0) * T))
            src, dst = out_vm.at[idx], out_hbm.at[idx]
        return pltpu.make_async_copy(src, dst, sems.at[_SEM_OF[item]])

    q_full, q_rows = {}, {}
    probs = {}
    attn = {}
    attn_lhs = {}
    acc = {}

    def qproj(g, heads, k0, k1, b0, b1):
        lhs = x_vm[b0 * SQ:b1 * SQ, k0 * T:k1 * T]
        for h in heads:
            col = g * GW + h * DH
            y = jnp.dot(lhs, wq_vm[k0 * T:k1 * T, col:col + DH], preferred_element_type=F32)
            if (b0, b1) == (0, B):
                if k0 != 0:
                    if (g, h) not in q_full:
                        q_full[g, h] = jnp.concatenate(
                            [q_rows.pop((g, h, b)) for b in range(B)], axis=0)
                    y = y + q_full[g, h]
                q_full[g, h] = y
            else:
                if k0 != 0 and (g, h) in q_full:
                    whole = q_full.pop((g, h))
                    for b in range(B):
                        q_rows[g, h, b] = whole[b * SQ:(b + 1) * SQ]
                for b in range(b0, b1):
                    part = y[(b - b0) * SQ:(b - b0 + 1) * SQ]
                    q_rows[g, h, b] = part if k0 == 0 else part + q_rows[g, h, b]

    def scores(g, b):
        def q_of(h):
            return q_full[g, h][b * SQ:(b + 1) * SQ] if (g, h) in q_full else q_rows[g, h, b]
        q = jnp.concatenate([q_of(h) for h in range(REP)], axis=0).astype(BF16)
        st = lax.dot_general(k_vm[b, g], q, _NT_DIMS, preferred_element_type=F32)
        m = jnp.max(st, axis=0, keepdims=True)
        e = jnp.exp2((st - m) * LOG2E_SCALE)
        inv = 1.0 / jnp.sum(e, axis=0, keepdims=True)
        probs[g, b] = (e * inv).astype(BF16).T

    def pv(g, b):
        o = jnp.dot(probs.pop((g, b)), v_vm[b, g], preferred_element_type=F32)
        for h in range(REP):
            attn[g, b, h] = o[h * SQ:(h + 1) * SQ]

    def out_lhs(g, b0, b1):
        if (g, b0, b1) not in attn_lhs:
            cols = [jnp.concatenate([attn[g, b, h] for b in range(b0, b1)], axis=0)
                    for h in range(REP)]
            attn_lhs[g, b0, b1] = jnp.concatenate(cols, axis=1).astype(BF16)
        return attn_lhs[g, b0, b1]

    def wo_tile(g, j):
        return wo_vm[g * GW:(g + 1) * GW, j * T:(j + 1) * T]

    def oproj(g, j):
        y = jnp.dot(out_lhs(g, 0, B), wo_tile(g, j), preferred_element_type=F32)
        acc[j] = y if j not in acc else y + acc[j]

    def ofinal(g, b0, b1, j0, j1):
        for j in range(j0, j1):
            y = jnp.dot(out_lhs(g, b0, b1), wo_tile(g, j), preferred_element_type=F32)
            total = y + acc[j][b0 * SQ:b1 * SQ]
            out_vm[b0 * SQ:b1 * SQ, j * T:(j + 1) * T] = total.astype(BF16)

    emit = {"start": lambda item: copy(item).start(), "wait": lambda item: copy(item).wait(),
            "qproj": qproj, "scores": scores, "pv": pv, "oproj": oproj, "ofinal": ofinal}
    for step in _SCHEDULE:
        emit[step[0]](*step[1:])


def _compiler_params():
    params = dict(vmem_limit_bytes=64 * 1024 * 1024)
    if jax.__version_info__ >= (0, 12):
        params.update(flags={"XLA_TPU_RESCHEDULE_DMA_DONES": True}, disable_semaphore_checks=True)
    return pltpu.CompilerParams(**params)


@jax.jit
def pallas_standalone__gqa_block_cached__near_ridge_kernel(
    x: jax.Array,
    k_cache: jax.Array,
    v_cache: jax.Array,
    wq: jax.Array,
    wo: jax.Array,
):
    assert x.shape == (B, SQ, D), x.shape
    assert k_cache.shape == v_cache.shape == (B, HKV, SK, DH), (k_cache.shape, v_cache.shape)
    assert wq.shape == (D, HQ * DH) and wo.shape == (HQ * DH, D), (wq.shape, wo.shape)

    any_space = pl.BlockSpec(memory_space=pl.ANY)
    out = pl.pallas_call(
        _kernel,
        in_specs=[any_space] * 5,
        out_specs=any_space,
        out_shape=jax.ShapeDtypeStruct((B * SQ, D), x.dtype),
        scratch_shapes=[
            pltpu.VMEM((B * SQ, D), x.dtype),
            pltpu.VMEM((B, HKV, SK, DH), k_cache.dtype),
            pltpu.VMEM((B, HKV, SK, DH), v_cache.dtype),
            pltpu.VMEM((D, HQ * DH), wq.dtype),
            pltpu.VMEM((HQ * DH, D), wo.dtype),
            pltpu.VMEM((B * SQ, D), x.dtype),
            pltpu.SemaphoreType.DMA((len(_COPIES),)),
        ],
        compiler_params=_compiler_params(),
    )(x.reshape(B * SQ, D), k_cache, v_cache, wq, wo)
    return out.reshape(B, SQ, D)
```
